```python
import os as _os
_os.environ.setdefault("JAX_PLATFORMS", "cpu")
import jax
import jax.numpy as jnp

def _softmax(x, axis=-1):
    return jax.nn.softmax(x, axis=axis)
def _gelu(x):
    return jax.nn.gelu(x, approximate=True)
def _silu(x):
    return jax.nn.silu(x)
def _sigmoid(x):
    return jax.nn.sigmoid(x)
def _layernorm(x, axis=-1, eps=1e-5):
    m = jnp.mean(x, axis=axis, keepdims=True)
    v = jnp.var(x, axis=axis, keepdims=True)
    return (x - m) / jnp.sqrt(v + eps)
def _scatter_add(tgt, idx, src, axis=0):
    return tgt.at[idx].add(src)
def _segment_sum(src, seg, n):
    return jax.ops.segment_sum(src, seg, n)
class _Rng:
    def __init__(self, key):
        self._k = key
    def _next(self):
        self._k, sub = jax.random.split(self._k)
        return sub
    def normal(self, shape):
        return jax.random.normal(self._next(), shape, dtype=jnp.bfloat16)
    def randint(self, lo, hi, shape):
        return jax.random.randint(self._next(), shape, lo, hi, dtype=jnp.int32)
    def uniform(self, shape, lo=0.0, hi=1.0):
        return jax.random.uniform(self._next(), shape, jnp.bfloat16, lo, hi)
    def permutation(self, n):
        return jax.random.permutation(self._next(), n)


kernel_name = 'gated_mix__linear_attn_block__swiglu_ffn__prompt'

def setup_inputs():
    _rng = _Rng(jax.random.key(int.from_bytes(__import__("os").urandom(4), "little")))
    _w = (lambda a: (lambda t: t.astype(jnp.bfloat16) if jnp.issubdtype(t.dtype, jnp.floating) else t)(jnp.asarray(a)))
    def _A_setup():
        B, S, D = 1, 2048, 512
        return {
            "x": _w((lambda *s: _rng.normal(s) * 0.05)(B, S, D)),
            "wqkv": _w((lambda *s: _rng.normal(s) * 0.8)(D, 3 * D)),
            "wo": _w((lambda *s: _rng.normal(s) * 0.05)(D, D)),
        }
    _A_in = _A_setup()

    def _B_setup():
        B, S, D, F = 1, 2048, 512, 1792
        return {
            "x": _w((lambda *s: _rng.normal(s) * 0.05)(B, S, D)),
            "w_gate": _w((lambda *s: _rng.normal(s) * 0.1)(D, F)),
            "w_up": _w((lambda *s: _rng.normal(s) * 0.1)(D, F)),
            "w_down": _w((lambda *s: _rng.normal(s) * 0.1)(F, D)),
        }
    _B_in = _B_setup()

    return {
        "A_x": _A_in["x"],
        "A_wqkv": _A_in["wqkv"],
        "A_wo": _A_in["wo"],
        "B_x": _B_in["x"],
        "B_w_gate": _B_in["w_gate"],
        "B_w_up": _B_in["w_up"],
        "B_w_down": _B_in["w_down"],
        "gate_w": _w((lambda *s: _rng.normal(s) * 0.05)(512) * 16.0),
    }

def reference(A_x, A_wqkv, A_wo, B_x, B_w_gate, B_w_up, B_w_down, gate_w):
    def _A_ref(x, wqkv, wo):
        B, S, D = x.shape
        H = 32; Dh = D // H
        qkv = (lambda x, *d: x.transpose(*d))((x @ wqkv).reshape(B, S, 3, H, Dh), 2, 0, 3, 1, 4)
        q, k, v = qkv[0], qkv[1], qkv[2]
        phi = lambda t: jnp.where(t > 0, t + 1, jnp.exp(t)) + 1e-6
        pq, pk = phi(q), phi(k)
        kv = jnp.einsum("bhsd,bhse->bhde", pk, v)
        z = jnp.einsum("bhsd->bhd", pk)
        num = jnp.einsum("bhqd,bhde->bhqe", pq, kv)
        den = jnp.einsum("bhqd,bhd->bhq", pq, z)[..., None] + 1e-6
        o = num / den
        return (lambda x, *d: x.transpose(*d))(o, 0, 2, 1, 3).reshape(B, S, D) @ wo

    def _B_ref(x, w_gate, w_up, w_down):
        g = _silu(x @ w_gate)
        u = x @ w_up
        return (g * u) @ w_down

    x = A_x
    g = _sigmoid((x * gate_w).sum(-1, keepdims=True))
    a = _A_ref(x, A_wqkv, A_wo)
    b = _B_ref(x, B_w_gate, B_w_up, B_w_down)
    return g * a + (1 - g) * b
```

```python
import itertools

import jax
import jax.numpy as jnp
from jax import lax
import jax.experimental.pallas as pl
import jax.experimental.pallas.tpu as pltpu

F32, BF16 = jnp.float32, jnp.bfloat16
T = 128
HEAD = 16
STEPS = 4

LHS = (((2, 1), (3, 1)), ((3, 1),), ((0, 1),), ((0, 1), (1, 1)),
       ((0, 1), (3, 1)), ((2, 1), (0, -1)), ((1, 1), (3, -1)))
RHS = (((0, 1),), ((2, 1), (0, -1)), ((1, 1), (3, -1)), ((3, 1),),
       ((0, 1), (3, 1)), ((0, 1), (1, 1)), ((2, 1), (3, 1)))
OUT = (((2, 1), (3, -1)), ((0, 1), (2, 1)), ((1, 1), (3, 1)), ((1, 1), (0, -1)),
       ((0, 1), (3, 1)), ((3, 1),), ((0, 1),))
FOLDED = (((0, 1),), ((3, 1),)) + OUT[:4]
NT = (((1,), (1,)), ((), ()))


def _mix(terms, quad):
    v = quad[terms[0][0]]
    for q, sign in terms[1:]:
        v = v + quad[q] if sign > 0 else v - quad[q]
    return v


def _spread(terms, vals, acc):
    for q, sign in terms:
        if acc[q] is None:
            acc[q] = sign, vals
        elif sign == acc[q][0]:
            acc[q] = sign, [a + v for a, v in zip(acc[q][1], vals)]
        else:
            acc[q] = 1, [v - a if sign > 0 else a - v for a, v in zip(acc[q][1], vals)]


def _gather(table, products):
    acc = [None] * 4
    for terms, m in zip(table, products, strict=True):
        _spread(terms, [m], acc)
    return [vals[0] for _, vals in acc]


def _encode(table, quadrant, put, src):
    blocks = {}
    for r in sorted(range(7), key=lambda r: (sum(q for q, _ in table[r] if q in (1, 2)), len(table[r]))):
        yield src
        new = [q for q, _ in table[r] if q not in blocks]
        if new:
            q = new[0]
            blocks[q] = quadrant(q)
        else:
            blocks[q][0] = quadrant(q)[0]
        quad = [_mix(table[r], {k: v[e] for k, v in blocks.items()}) for e in range(4)]
        put(r, [_mix(terms, quad) for terms in table])


def _decode(table, product, finish, src, order=range(7)):
    acc = [None] * 4
    for n, r in enumerate(order):
        yield src
        _spread(table[r], product(r), acc)
        for q, _ in table[r]:
            if all(q != q2 for r2 in order[n + 1:] for q2, _ in table[r2]):
                finish(q, acc[q][1])
                yield None


def _stack(values):
    return jnp.concatenate([v[None] for v in values], axis=0)


def _by_column(blocks):
    return [blocks[0], blocks[2], blocks[1], blocks[3]]


def _phi(t):
    return jnp.where(t > 0, t + 1.0, jnp.exp(t)) + 1e-6


def _dot(a, b, dims=(((1,), (0,)), ((), ()))):
    return lax.dot_general(a, b, dims, preferred_element_type=F32)


def _divmod(i, n):
    return divmod(i, n) if isinstance(i, int) else (lax.div(i, n), lax.rem(i, n))


def _tile(i, n=1):
    return pl.ds(i * T, n * T)


def _kernel(x_hbm, wqkv_hbm, wo_hbm, wg_hbm, wu_hbm, wd_hbm, gw_hbm, o_hbm,
            x_v, wq_v, wk_v, wv_v, wo_v, wu_v, wd_v, gw_v,
            xs, ops, ds, dl, gb, kvb, tr, zacc, zrow, bal, sg, hh, hq, small, prod, sems, bar):
    D = o_hbm.shape[2]
    F = wd_hbm.shape[0]
    NB = o_hbm.shape[0] // 4
    NC = F // (2 * T)
    heads = D // HEAD
    step = pl.program_id(0)
    zero = lax.shift_right_logical(step, 8)

    PS, WS, WT, HL = 196, 392, 392 + 49 * NC, 0
    p_u = lambda j: lambda b: 42 * (4 * {5: 1, 6: 4}.get(j, j) + b)
    p_k = lambda b: 42 * (4 + b)
    p_q = lambda b: 42 * (8 + 2 * b)
    p_o = lambda b: 84 * b
    P_G, P_M = 0, 84

    halves = lambda src, dst, n: [(src.at[pl.ds(i * n, n)], dst.at[pl.ds(i * n, n)]) for i in range(2)]
    x_part = lambda lo, n: halves(x_hbm.at[pl.ds(lo, n)], x_v.at[pl.ds(lo, n), :T], n // 2)
    sources = dict(
        x0=x_part(0, 2), x0b=x_part(2, 2), x1=x_part(4, 4), x2=x_part(8, 8),
        wk=halves(wqkv_hbm.at[:, D:2 * D], wk_v.at[0], D // 2), wq=[(wqkv_hbm.at[:, :D], wq_v.at[0, :D])],
        wv=[(wqkv_hbm.at[:, 2 * D:], wv_v)], wo=[(wo_hbm, wo_v)], wd=[(wd_hbm, wd_v.at[0, :F])], gw=[(gw_hbm, gw_v)])

    def inputs(*names):
        for name in names:
            if isinstance(name, str):
                pairs, sem = sources[name], 2 * list(sources).index(name)
            else:
                start = 2 * T * name if isinstance(name, int) else pl.multiple_of(2 * T * name, 2 * T)
                pairs = [(w.at[:, pl.ds(start, 2 * T)], wu_v.at[2 * name + n, :D]) for n, w in enumerate((wg_hbm, wu_hbm))]
                sem = 2 * (len(sources) + name)
            for n, (src, dst) in enumerate(pairs):
                yield pltpu.make_async_copy(src, dst, sems.at[sem + n])

    def wait(*names):
        for copy in inputs(*names):
            copy.wait()

    def tick(ref, value):
        n = 16 if ref.dtype == BF16 else 8
        ref[zero, ref.shape[1] - n:, :T] = value[:n].astype(ref.dtype)

    def run(waves, tasks=()):
        rounds = list(itertools.zip_longest(waves, tasks, fillvalue=(None, 0, 0, 0)))
        assert len(waves) in (0, len(rounds))
        while rounds:
            (wave, w0, *_), (task, t0, slabs, steps) = rounds[0]
            count = next((n for n, (w, t) in enumerate(rounds)
                          if w[:2] + t[:3] != (wave, w0 + n * bool(wave), task, t0 + n * slabs, slabs)), len(rounds))
            rounds = rounds[count:]

            def body(i, carry):
                outs = [(ref, slot, _stack(vs)) for ref, slot, vs in wave(w0 + i)] if wave else []
                work = itertools.chain.from_iterable(task(t0 + i * slabs + n) for n in range(slabs))
                if not (task and outs):
                    for ref, slot, v in outs:
                        ref[pl.ds(slot, len(v)), :T, :] = v
                    list(work)
                    return carry
                src = next(work)
                for n in range(8):
                    for ref, slot, v in outs:
                        ref[pl.ds(slot, len(v)), 16 * n:16 * n + 16, :] = v[:, 16 * n:16 * n + 16]
                    ticked = False
                    for _ in range(-(-n * slabs * steps // 8), -(-(n + 1) * slabs * steps // 8)):
                        if src is not None and not ticked:
                            tick(src, outs[-1][2][-1, 16 * n:16 * n + 16])
                            ticked = True
                        src = next(work, False)
                assert src is False
                return carry

            if count == 1:
                body(0, 0)
            else:
                lax.fori_loop(0, count, body, 0, unroll=True)

    def over(task, lo, hi, slabs=1, steps=7):
        return [(task, t, slabs, steps) for t in range(lo, hi, slabs)]

    idle = [(None, 0, 0, 0)]

    def store(ref, r0, row):
        def put(r, vs):
            ref[pl.ds(r0 + 7 * r, 7), pl.ds(row, vs[0].shape[0]), :] = _stack(vs).astype(BF16)
        return put

    def load(ref, slot, count, rows):
        v = ref[pl.ds(slot, count), rows, :]
        return [v[e] for e in range(count)]

    quadrants = lambda get: lambda q: [get(q // 2 * 2 + e // 2, q % 2 * 2 + e % 2).astype(F32) for e in range(4)]
    stored = lambda ref, slot, rows: lambda q: _by_column(load(ref, slot + 8 * (q % 2) + 4 * (q // 2), 4, rows))

    def transposed(w_v):
        def task(k):
            for j in range(4):
                yield w_v
                tr[k, _tile(j), :] = w_v[0, _tile(k), _tile(j)].astype(F32).T
        return over(task, 0, 4, 1, 4)

    def k_weights(t):
        return _encode(RHS, quadrants(lambda k, j: tr[k, pl.ds(j * T + 16 * t, 16), :]), store(ops, WT, 16 * t), tr)

    def dim_major(t):
        d, h = _divmod(t, 2)
        for k in range(4):
            for j in range(4):
                yield tr
                hq[4 * k + j, pl.ds(16 * t, 16), :] = tr[k, pl.ds(h * 16 * HEAD + 4 * j + d, 16, stride=HEAD), :]

    def q_weights(t):
        return _encode(RHS, quadrants(lambda k, j: hq[4 * k + j, pl.ds(16 * t, 16), :]), store(ops, WT, 16 * t), hq)

    def balance():
        size = []
        for n in range(2):
            v = sum(jnp.abs(wu_v[n, s:s + 16, :].astype(F32)) for s in range(0, D, 64))
            v = jnp.sum(v[:, :T] + v[:, T:], axis=0, keepdims=True)
            size.append(jnp.broadcast_to(jnp.sum(v, axis=1, keepdims=True), (16, T)) + 1e-30)
        scale = jnp.clip(size[1] / size[0], 2.0 ** -30, 2.0 ** 30)
        bal[0] = scale
        bal[1] = 0.5 / scale

    def gu_weights(w, j, dst):
        def task(t):
            def get(k, n):
                v = w[2 * j + n % 2, pl.ds(k * T + 16 * t, 16), _tile(n // 2)]
                return v if n % 2 else v.astype(F32) * bal[0]
            return _encode(RHS, quadrants(get), store(dst, WS + 49 * j, 16 * t), wu_v)
        return task

    def d_weights(t):
        kb, s = _divmod(t, 8)
        return _encode(RHS, quadrants(lambda k, n: wd_v[0, pl.ds((4 * kb + k) * T + 16 * s, 16), _tile(n)]),
                       store(ds, 0, 16 * t), wd_v)

    def m_weights(t):
        d, h = _divmod(t, 2)
        get = lambda k, n: jnp.concatenate([prod[P_M + 8 * h + 4 * i + n, pl.ds(8 * (4 * k + d), 8), :] for i in range(2)], axis=0)
        return _encode(RHS, quadrants(get), store(ds, 0, 3 * T + 16 * t), prod)

    def l_weights(t):
        for n in range(2):
            yield wd_v
            quad = [wd_v[0, pl.ds(F - (2 - q // 2) * T + 16 * t, 16), _tile(q % 2 * 2 + n)].astype(F32) for q in range(4)]
            store(dl, 0, 16 * t)(n, [_mix(terms, quad) for terms in RHS])

    def x_rows(t):
        b, s = _divmod(t, 8)
        return lambda i, k: x_v[4 * b + i, pl.ds(16 * s, 16), _tile(k)]

    def x_sums(t):
        return _encode(LHS, quadrants(x_rows(t)), store(xs, 0, 16 * t), x_v)

    def first_x_sums(groups):
        quadrant = quadrants(lambda i, k: x_v[i, :T, _tile(k)])
        for r in groups:
            blocks = {q: quadrant(q) for q, _ in LHS[r]}
            quad = [_mix(LHS[r], {q: v[e] for q, v in blocks.items()}) for e in range(4)]
            store(xs, 0, 0)(r, [_mix(terms, quad) for terms in LHS])

    def gates(t):
        b, s = _divmod(t, 8)
        gw = gw_v[...].astype(F32).reshape(1, D)
        for i in range(4):
            yield x_v
            v = [x_rows(t)(i, k).astype(F32) * gw[:, k * T:(k + 1) * T] for k in range(4)]
            v = jnp.broadcast_to(jnp.sum((v[0] + v[1]) + (v[2] + v[3]), axis=1, keepdims=True), (16, T))
            sg[4 * b + i, pl.ds(16 * s, 16), :] = 0.5 - 0.5 * jnp.tanh(0.5 * v)

    def projection(p, slot, rows, finish):
        product = lambda r: _gather(FOLDED, load(p, slot + 3 * r, 3, rows) + load(p, slot + 21 + 3 * r, 3, rows))
        return _decode(OUT, product, finish, prod)

    def k_post(t):
        b, s = _divmod(t, 16)

        def finish(q, c):
            hh[pl.ds(48 * b + 32 + 8 * (q % 2) + 4 * (q // 2), 4), pl.ds(8 * s, 8), :] = _phi(_stack(_by_column(c)))
        return projection(prod, p_k(b), pl.ds(8 * s, 8), finish)

    def k_sums(h, dst, z):
        def task(t):
            def put(r, vs):
                store(dst, PS, 16 * t)(r, vs)
                if r in (1, 2):
                    for j in range(2):
                        z[pl.ds((2 * (r - 1) + j) * T + 16 * t, 16), :] = vs[1 + j]
            return _encode(OUT, stored(h, 32, pl.ds(16 * t, 16)), put, hh)
        return task

    def z_total(d):
        for part in range(4):
            yield zacc
            z = [zacc[b, pl.ds(part * T + d, 8, stride=HEAD), :] for b in range(NB)]
            tr[0, pl.ds(d * heads + 8 * part, 8), :] = sum(z[1:], z[0])

    def z_rows(k):
        yield tr
        zrow[k] = jnp.broadcast_to(jnp.sum(tr[0, _tile(k), :].T, axis=0, keepdims=True), (8, T))

    def g_post(t):
        rows = pl.ds(16 * t, 16)

        def finish(q, c):
            for e in range(4):
                gb[4 * (q % 2 * 2 + e % 2) + q // 2 * 2 + e // 2, rows, :] = c[e].astype(BF16)
        return _decode(RHS, lambda r: _gather(RHS, load(prod, P_G + 7 * r, 7, rows)), finish, prod, (1, 6, 2, 5, 0, 3, 4))

    def kv_post(j):
        row, col = [lax.broadcasted_iota(jnp.int32, (16, T), axis) for axis in range(2)]
        for d in range(0, HEAD, 2):
            yield small
            v = jnp.concatenate([small[j, pl.ds(d + e, 8, stride=HEAD), :] for e in range(2)], axis=0)
            kvb[j, 8 * d:8 * d + 16, :] = jnp.where((row & 7) == (col >> 4), v, 0.0).astype(BF16)

    def q_post(p, b):
        def task(t):
            rows, half = pl.ds(8 * t, 8), {}

            def finish(q, c):
                a = [_phi(v) for v in c]
                hq[pl.ds(8 * (q % 2) + 4 * (q // 2), 4), rows, :] = _stack(_by_column(a))
                z = load(zrow, q % 2 * 2, 2, slice(None))
                for n in range(2):
                    i, v = q // 2 * 2 + n, a[2 * n] * z[0] + a[2 * n + 1] * z[1]
                    if i in half:
                        v = v + half[i]
                        hq[16 + i, rows, :] = (v + pltpu.roll(v, 32, 1)) + (pltpu.roll(v, 64, 1) + pltpu.roll(v, 96, 1))
                    half[i] = v
            return projection(p, p_q(b), rows, finish)
        return over(task, 0, 16, 1, 11)

    def q_norm(g, b):
        def task(t):
            n, s = _divmod(t, 8)
            rows = pl.ds(16 * s, 16)
            yield hq
            small[pl.ds(2 * n, 2), rows, :] = (1.0 - g[pl.ds(4 * b + 2 * n, 2), rows, :]) / (hq[pl.ds(16 + 2 * n, 2), rows, :] + 1e-6)
        return task

    def q_sums(dst, b):
        def task(t):
            rows = pl.ds(16 * t, 16)

            def quadrant(q):
                scale = load(small, q // 2 * 2, 2, rows)
                return [v * scale[e // 2] for e, v in enumerate(stored(hq, 0, rows)(q))]
            return _encode(LHS, quadrant, store(dst, 196 * b + 147, 16 * t), hq)
        return task

    def swiglu(p, j, t, put):
        b, s = _divmod(t, 16)
        rows = pl.ds(8 * s, 8)

        def finish(q, c):
            half = bal[1:, :8, :] * _stack(c[::2])
            m = half * _stack(c[1::2]) * sg[pl.ds(4 * b + q // 2 * 2, 2), rows, :]
            put(b, rows, q, m + m * jnp.tanh(half))
        return projection(p, p_u(j)(b), rows, finish)

    def gu_post(p, h, j):
        def put(b, rows, q, v):
            h[pl.ds(48 * b + 8 * j + 2 * q, 2), rows, :] = v
        return over(lambda t: swiglu(p, j, t, put), 0, 16 * NB, 2, 11)

    def h_sums(h, dst, b):
        def task(t):
            kb, s = _divmod(t, 8)
            return _encode(LHS, stored(h, 48 * b + 16 * kb, pl.ds(16 * s, 16)), store(dst, 196 * b + 49 * kb, 16 * s), hh)
        return task

    def l_sums(t):
        b, s = _divmod(t, 8)
        out = [{}, {}]
        for n in range(2):
            yield from swiglu(prod, NC - 1, 2 * t + n, lambda b, rows, q, v: out[n].update({q: v}))
        for i in range(2):
            quad = [jnp.concatenate([o[q][i] for o in out], axis=0) for q in range(4)]
            store(ops, HL + 14 * b, 16 * s)(i, [_mix(terms, quad) for terms in LHS])
            yield None

    def o_post(b, order=range(7), resume=(), suspend=()):
        def task(t):
            rows = pl.ds(16 * t, 16)

            def product(r):
                return [c + v for c, v in zip(_gather(OUT, load(prod, p_o(b) + 7 * r, 7, rows)),
                                              load(prod, p_o(b) + 49 + 4 * r, 4, rows))]

            def finish(q, c):
                if q in suspend:
                    hq[pl.ds(4 * q, 4), rows, :] = _stack(c)
                    return
                if q in resume:
                    c = [a + v for a, v in zip(c, load(hq, 4 * q, 4, rows))]
                for n in range(2):
                    x_v[4 * b + q // 2 * 2 + n, rows, _tile(q % 2 * 2, 2)] = jnp.concatenate(c[2 * n:2 * n + 2], axis=1).astype(BF16)
            return _decode(OUT, product, finish, prod, order)
        return task

    def project(p, slot, product, lo, hi):
        def fold(w):
            r, b = _divmod(w, hi - lo)
            m4, m5, m6, m0 = [product(7 * r + e, lo + b) for e in (4, 5, 6, 0)]
            return [(p, slot(lo + b) + 3 * r, [m4 + m6, m4 + m5, m0])]

        def four(w):
            n, b = _divmod(w, hi - lo)
            return [others(p, slot, product, 4 * n, 4, lo + b)]
        return waves(fold, 7 * (hi - lo)) + waves(four, 5 * (hi - lo))

    def others(p, slot, product, n, count, b):
        return p, slot(b) + 21 + n, [product(7 * r + 1 + e, b) for r, e in [_divmod(n + k, 3) for k in range(count)]]

    def project_all(p, slot, product):
        return project(p, slot, product, 0, NB) + waves(lambda w: [others(p, slot, product, 20, 1, b) for b in range(NB)], 1)

    waves = lambda wave, count: [(wave, w) for w in range(count)]
    wide = lambda ref, r, stride: jnp.concatenate([ref[r + k * stride] for k in range(4)], axis=1)
    k_dot = lambda r, b: _dot(ops[WT + r], xs[r, _tile(b), :], NT)
    q_dot = lambda r, b: _dot(xs[r, _tile(b), :], ops[WT + r], NT)
    u_dot = lambda w, j: lambda r, b: _dot(xs[r, _tile(b), :], w[WS + 49 * j + r])
    o_dot = lambda w, b, r: _dot(wide(w, 196 * b + r, 49), ds[r])

    @pl.when(step == 0)
    def _():
        for copy in inputs(0, "x0", "x0b", "x1", "wk", "x2", 1, "gw", *range(2, NC), "wq", "wd", "wv", "wo"):
            copy.start()
        for ref in (xs, ds, dl, gb, kvb, zrow, bal, sg):
            tick(ref, jnp.zeros((16, T), F32))
        keys = lambda b: project(prod, p_k, k_dot, b, b + 1)
        first = lambda lo, hi: project(prod, p_u(0), u_dot(ops, 0), lo, hi)
        last = lambda lo: waves(lambda w: [others(prod, slot, dot, 20, 1, b) for b in (lo, lo + 1)
                                           for slot, dot in ((p_k, k_dot), (p_u(0), u_dot(ops, 0)))], 1)
        u0, u1 = first(0, 1), first(1, 2)
        wait(0)
        balance()
        run([], over(gu_weights(wu_v, 0, ops), 0, 8))
        wait("x0")
        first_x_sums((2, 3))
        run(u0[2:4] + u0[9:10])
        wait("x0b")
        first_x_sums((1, 0, 4, 5, 6))
        run(u0[1:2] + u0[8:9] + u0[7:8] + u0[10:])
        wait("x1")
        run(u0[:1] + u0[4:7], over(x_sums, 8, 16, 2))
        wait("wk")
        run([], transposed(wk_v))
        run(u1[7:] + u1[:7], 3 * idle + over(k_weights, 0, 8))
        wait("x2")
        run(last(0) + keys(0) + keys(1), over(x_sums, 16, 32) + over(k_post, 0, 16, 2, 11))
        wait(1, "gw")
        run(last(2) + keys(2) + keys(3) + first(2, 4),
            over(gu_weights(wu_v, 1, ops), 0, 8) + over(k_post, 16, 48, 2, 11) + over(gates, 0, 32, 2, 4)
            + over(k_post, 48, 64, 2, 11))

    p, w = prod.at[pl.ds(168 * step, 336)], ops.at[pl.ds(49 * step, WS + 147)]
    wait(step + 2)
    run(project_all(p, p_u(1), u_dot(w, 1)),
        over(k_sums(hh.at[pl.ds(48 * step, 48)], w, zacc.at[step]), 0, 8)
        + over(gu_weights(wu_v.at[pl.ds(2 * step, 6)], 2, w), 0, 8) + gu_post(p, hh.at[pl.ds(8 * step, 152)], 0))

    @pl.when(step == STEPS - 1)
    def _():
        wait(6, "wq", "wd")
        run(waves(lambda r: [(prod, P_G + r, [_dot(wide(ops, PS + r, 49), xs[r])])], 49) + project_all(prod, p_u(5), u_dot(ops, 5)),
            transposed(wq_v) + idle + over(lambda t: [tr], 0, 1, 1, 1) + over(gu_weights(wu_v, 6, ops), 0, 8)
            + over(dim_major, 0, 8, 1, 16) + over(d_weights, 0, 24) + over(q_weights, 0, 8) + over(l_weights, 0, 8, 4, 2)
            + over(g_post, 0, 8, 1, 11) + gu_post(prod, hh, 4))
        wait("wv", "wo")
        kv = [(lambda w, j=j: [(small, j, [_dot(wide(gb, 4 * j, 1), wv_v[:, _tile(j)])])], 0) for j in range(4)]
        mixed = waves(lambda j: [(prod, P_M + 4 * j, [_dot(kvb[j], wo_v[_tile(j), _tile(n)]) for n in range(4)])], 4)
        run(kv + project_all(prod, p_q, q_dot) + mixed + project_all(prod, p_u(6), u_dot(ops, 6)),
            over(z_total, 0, 16, 4, 4) + over(h_sums(hh, ops, 0), 0, 16) + over(kv_post, 0, 4, 2, 8)
            + over(z_rows, 0, 4, 2, 1) + gu_post(prod, hh, 5) + idle + q_post(prod, 0) + over(m_weights, 0, 8)
            + over(h_sums(hh, ops, 0), 16, 24) + over(q_norm(sg, 0), 0, 16, 2, 1) + over(q_sums(ops, 0), 0, 8))

        def rows_out(b, carry):
            p, w, h = prod.at[pl.ds(84 * b, 504)], ops.at[pl.ds(196 * b, 392)], hh.at[pl.ds(48 * b, 96)]
            sums, norm = h_sums(h, w, 1), q_norm(sg.at[pl.ds(4 * b, 8)], 1)
            run(waves(lambda r: [(p, r, [o_dot(w, 0, r)])], 49),
                q_post(p, 1) + over(sums, 16, 24) + over(lambda t: itertools.chain(norm(t), sums(t)), 0, 16, 1, 8)
                + over(q_sums(w, 1), 0, 8))
            return carry

        end = NB - 1
        lax.fori_loop(0, end, rows_out, 0)
        main = waves(lambda r: [(prod, p_o(end) + r, [o_dot(ops, end, r)])], 46)
        run(main[:33], over(l_sums, 0, 8 * NB, 1, 24))
        pl.semaphore_signal(bar)
        pl.semaphore_wait(bar)

        sent = []

        def send(*window):
            sent.append(pltpu.make_async_copy(x_v.at[window], o_hbm.at[window], sems.at[len(sent)]))
            sent[-1].start()

        def leftover(w):
            b, r = _divmod(w, 7)
            return [(prod, p_o(b) + 49 + 4 * r, [_dot(ops[HL + 14 * b + 7 * (e // 2) + r], dl[7 * (e % 2) + r]) for e in range(4)])]

        tail = waves(leftover, 7 * NB) + main[33:]
        run(tail[:7])
        for n in range(2 * end):
            run(tail[7 + 4 * n:11 + 4 * n], over(o_post(n // 2), n % 2 * 4, n % 2 * 4 + 4, 1, 11))
            send(pl.ds(n // 2 * 4, 4), pl.ds(n % 2 * T // 2, T // 2))
        for n in range(2):
            run(tail[31 + 4 * n:35 + 4 * n], over(o_post(end, range(5), (), (0, 3)), 4 * n, 4 * n + 4, 1, 9))
            for i in range(4):
                send(4 * end + i, pl.ds(n * T // 2, T // 2), _tile(2 - i // 2 * 2, 2))
        run(tail[39:], over(o_post(end, [5], (3,)), 0, 8, 4, 2))
        for i in (2, 3):
            send(4 * end + i, _tile(0), _tile(2, 2))
        acc = [(1, [a + v]) for a, v in zip(load(hq, 0, 4, _tile(0)), load(prod, p_o(end) + 73, 4, _tile(0)))]
        for terms, m in zip(OUT, load(prod, p_o(end) + 42, 4, _tile(0)) + [o_dot(ops, end, r) for r in range(46, 49)]):
            _spread(terms, [m], acc)
        for e in (1, 2, 3, 0):
            x_v[4 * end + e // 2, :T, _tile(e % 2)] = acc[e][1][0].astype(BF16)
            send(4 * end + e // 2, _tile(0), _tile(e % 2))
        for copy in sent:
            copy.wait()


@jax.jit
def pallas_gated_mix__linear_attn_block__swiglu_ffn__prompt_kernel(
    A_x: jax.Array,
    A_wqkv: jax.Array,
    A_wo: jax.Array,
    B_x: jax.Array,
    B_w_gate: jax.Array,
    B_w_up: jax.Array,
    B_w_down: jax.Array,
    gate_w: jax.Array,
):
    del B_x
    B, S, D = A_x.shape
    F = B_w_gate.shape[1]
    assert (B, S, D, F) == (1, 2048, 512, 1792)
    bf = lambda *shape: pltpu.VMEM(shape, BF16)
    fp = lambda *shape: pltpu.VMEM(shape, F32)
    out = pl.pallas_call(
        _kernel,
        grid=(STEPS,),
        in_specs=[pl.BlockSpec(memory_space=pl.ANY)] * 7,
        out_specs=pl.BlockSpec(memory_space=pl.ANY),
        out_shape=jax.ShapeDtypeStruct((S // T, T, D), A_x.dtype),
        scratch_shapes=[
            bf(S // T, T + 16, D), bf(1, D + 16, D), bf(1, D + 16, D), bf(D, D), bf(D, D),
            bf(F // T, D + 16, 2 * T), bf(1, F + 16, D), bf(D),
            bf(49, S // 4, T), bf(4 * 196, T, T), bf(49, 4 * T, T), bf(14, T, T), bf(16, T, T), bf(4, T, T),
            fp(4, D + 24, T), fp(4, D + 24, T), fp(4, 8, T), fp(2, 16, T), fp(16, T + 8, T), fp(4 * 48, T + 8, T),
            fp(20, T + 8, T), fp(4, T + 24, T), fp(20 * 42, T + 8, T),
            pltpu.SemaphoreType.DMA((20 + F // T,)), pltpu.SemaphoreType.REGULAR,
        ],
        compiler_params=pltpu.CompilerParams(
            dimension_semantics=("arbitrary",), vmem_limit_bytes=126 * 1024 * 1024,
            disable_semaphore_checks=True),
    )(A_x.reshape(S // T, T, D), A_wqkv, A_wo, B_w_gate, B_w_up, B_w_down, gate_w)
    return out.reshape(B, S, D)
```
